```python
import os as _os
_os.environ.setdefault("JAX_PLATFORMS", "cpu")
import jax
import jax.numpy as jnp

def _softmax(x, axis=-1):
    return jax.nn.softmax(x, axis=axis)
def _gelu(x):
    return jax.nn.gelu(x, approximate=True)
def _silu(x):
    return jax.nn.silu(x)
def _sigmoid(x):
    return jax.nn.sigmoid(x)
def _layernorm(x, axis=-1, eps=1e-5):
    m = jnp.mean(x, axis=axis, keepdims=True)
    v = jnp.var(x, axis=axis, keepdims=True)
    return (x - m) / jnp.sqrt(v + eps)
def _scatter_add(tgt, idx, src, axis=0):
    return tgt.at[idx].add(src)
def _segment_sum(src, seg, n):
    return jax.ops.segment_sum(src, seg, n)
class _Rng:
    def __init__(self, key):
        self._k = key
    def _next(self):
        self._k, sub = jax.random.split(self._k)
        return sub
    def normal(self, shape):
        return jax.random.normal(self._next(), shape, dtype=jnp.bfloat16)
    def randint(self, lo, hi, shape):
        return jax.random.randint(self._next(), shape, lo, hi, dtype=jnp.int32)
    def uniform(self, shape, lo=0.0, hi=1.0):
        return jax.random.uniform(self._next(), shape, jnp.bfloat16, lo, hi)
    def permutation(self, n):
        return jax.random.permutation(self._next(), n)


kernel_name = 'standalone__cross_network_dcn_v2__recsys'

def setup_inputs():
    _rng = _Rng(jax.random.key(int.from_bytes(__import__("os").urandom(4), "little")))
    _w = (lambda a: (lambda t: t.astype(jnp.bfloat16) if jnp.issubdtype(t.dtype, jnp.floating) else t)(jnp.asarray(a)))
    B, F, D, L = 16384, 26, 16, 6
    Din = min(F * D, 512)
    R = max(Din // 4, 2)
    sc = Din ** -0.5
    return {
        "x0": _w((lambda *s: _rng.normal(s) * 0.05)(B, Din)),
        "U":  _w((lambda *s: _rng.normal(s) * 1.6)(L, Din, R) * sc),
        "V":  _w((lambda *s: _rng.normal(s) * 1.6)(L, R, Din) * sc),
        "bs": _w((lambda *s: _rng.normal(s) * 0.05)(L, Din)),
    }

def reference(x0, U, V, bs):
    x = x0
    for l in range(U.shape[0]):
        h = jnp.einsum('rd,bd->br', V[l], x)
        h = jnp.einsum('dr,br->bd', U[l], h)
        x = x0 * (h + bs[l]) + x
    return x
```

```python
import functools
import jax, jax.numpy as jnp
from jax import lax
from jax.experimental import pallas as pl
from jax.experimental.pallas import tpu as pltpu

F32 = jnp.float32
BF16 = jnp.bfloat16
U32 = jnp.uint32

def pk(x):
    return pltpu.bitcast(x, U32)
def upk(x):
    return pltpu.bitcast(x, BF16)

def _make(bt=1024, skew=3, usex0f=True, tail_split=4, ntail=4, xw="f32", zw="f32", nobc=True):
    ncb = bt // 128
    cw = 128
    def kernel(x_hbm, u_hbm, v_hbm, b_hbm, o_hbm, xbuf, obuf, u_ref, v_ref, b_ref,
               uz_ref, vm_ref, vb_ref, x0f_ref, xf_ref, wsem, xsem, osem):
        L, D, R = u_ref.shape
        B = x_hbm.shape[1]
        nchunk = B // bt
        KM = (D // 128) * 128
        KR = D - KM
        NZ = 128 - R - 1
        NL = KR - NZ

        def x_copy(i, slot):
            return pltpu.make_async_copy(x_hbm.at[:, pl.ds(pl.multiple_of(i * bt, bt), bt)], xbuf.at[slot], xsem.at[slot])
        def o_copy(i, slot):
            return pltpu.make_async_copy(obuf.at[slot], o_hbm.at[:, pl.ds(pl.multiple_of(i * bt, bt), bt)], osem.at[slot])

        v_cp = pltpu.make_async_copy(v_hbm, v_ref, wsem.at[0])
        u_cp = pltpu.make_async_copy(u_hbm, u_ref, wsem.at[1])
        b_cp = pltpu.make_async_copy(b_hbm, b_ref, wsem.at[2])
        v_cp.start(); b_cp.start(); u_cp.start()
        x_copy(0, 0).start()

        row = lax.broadcasted_iota(jnp.int32, (R, 128), 0)
        col = lax.broadcasted_iota(jnp.int32, (R, 128), 1)
        rk = lax.broadcasted_iota(jnp.int32, (128, 128), 0)
        ck = lax.broadcasted_iota(jnp.int32, (128, 128), 1)

        v_cp.wait()
        for l in range(L):
            v0 = v_ref[l, :, 0:128]
            vf = v_ref[l].astype(F32)
            for kt in range(KM // 128):
                vm_ref[l, kt] = vf[:, KR + kt * 128: KR + (kt + 1) * 128]
            for k in range(NL):
                e = jnp.where(rk == k, 1.0, 0.0).astype(BF16)
                vb_ref[l, k] = jnp.dot(v0, e, preferred_element_type=F32)
        b_cp.wait()
        u_cp.wait()
        sel = jnp.where((ck == rk + (R - 8)) & (rk >= NL) & (rk < KR), 1.0, 0.0).astype(BF16)
        bmat = b_ref[...]
        rl = lax.broadcasted_iota(jnp.int32, (L, 128), 0)
        cl = lax.broadcasted_iota(jnp.int32, (L, 128), 1)
        for l in range(L):
            v0 = v_ref[l, :, 0:128]
            w = jnp.dot(v0, sel, preferred_element_type=F32)
            w = jnp.where(row == col, 1.0, w).astype(BF16)
            uz = jnp.dot(u_ref[l], w, preferred_element_type=F32)
            e = jnp.where((rl == l) & (cl == R), 1.0, 0.0).astype(BF16)
            uz = uz + lax.dot_general(bmat, e, (((0,), (0,)), ((), ())), preferred_element_type=F32)
            uz_ref[l] = pk(uz.astype(BF16))

        sub = lax.broadcasted_iota(jnp.int32, (8, cw), 0)

        def cs(c):
            return slice(c * cw, (c + 1) * cw)

        def body(i, carry):
            slot = lax.rem(i, 2)
            x_copy(i, slot).wait()
            @pl.when(i + 1 < nchunk)
            def _():
                x_copy(i + 1, 1 - slot).start()
            @pl.when(i >= 2)
            def _():
                o_copy(i - 2, slot).wait()
            x0_ref = xbuf.at[slot]
            o_ref = obuf.at[slot]
            zs = {}

            def x0rows(c, r0, r1):
                if usex0f:
                    return x0f_ref[c, r0:r1, :]
                return x0_ref[r0:r1, cs(c)].astype(F32)

            def stage_mm1(l, c):
                src = x0f_ref if l == 0 else xf_ref
                acc = None
                for k in range(NL):
                    t = vb_ref[l, k] * src[c, k:k + 1, :]
                    acc = t if acc is None else acc + t
                for kt in range(KM // 128):
                    r0 = KR + kt * 128
                    if l == 0:
                        xb = x0_ref[r0:r0 + 128, cs(c)]
                    else:
                        xb = xf_ref[c, r0:r0 + 128, :]
                        if xw == "bf16":
                            xb = xb.astype(BF16)
                    acc = acc + jnp.dot(vm_ref[l, kt], xb, preferred_element_type=F32)
                first = jnp.where(sub == 0, 1.0, src[c, 8:16, :])
                z = jnp.concatenate([acc, first, src[c, 16:32, :]], axis=0)
                zs[c] = z.astype(BF16) if zw == "bf16" else z

            def stage_mm2(l, c, nsplit=1):
                bounds = [((D // 16) * j // nsplit) * 16 for j in range(nsplit + 1)]
                for r0, r1 in zip(bounds[:-1], bounds[1:]):
                    y = jnp.dot(upk(uz_ref[l, r0 // 2:r1 // 2, :]), zs[c], preferred_element_type=F32)
                    x0 = x0rows(c, r0, r1)
                    x = x0 if l == 0 else xf_ref[c, r0:r1, :]
                    xn = x0 * y + x
                    if l == L - 1:
                        o_ref[r0:r1, cs(c)] = xn.astype(BF16)
                    else:
                        xf_ref[c, r0:r1, :] = xn

            total = L * ncb
            for t in range(0, total + skew):
                if t < total:
                    l, c = divmod(t, ncb)
                    if l == 0:
                        if usex0f:
                            x0f_ref[c] = x0_ref[:, cs(c)].astype(F32)
                        else:
                            x0f_ref[c, 0:KR, :] = x0_ref[0:KR, cs(c)].astype(F32)
                    stage_mm1(l, c)
                if 0 <= t - skew < total:
                    l, c = divmod(t - skew, ncb)
                    stage_mm2(l, c, tail_split if t - skew >= total - ntail else 1)
            o_copy(i, slot).start()
            return carry

        lax.fori_loop(0, nchunk, body, 0)
        if nchunk >= 2:
            o_copy(nchunk - 2, (nchunk - 2) % 2).wait()
        o_copy(nchunk - 1, (nchunk - 1) % 2).wait()

    def fn(x0, U, V, bs):
        B, D = x0.shape
        L, _, R = U.shape
        xt = x0.T
        out = pl.pallas_call(
            kernel,
            in_specs=[pl.BlockSpec(memory_space=pl.ANY)] * 4,
            out_specs=pl.BlockSpec(memory_space=pl.ANY),
            out_shape=jax.ShapeDtypeStruct(xt.shape, x0.dtype),
            scratch_shapes=[pltpu.VMEM((2, D, bt), BF16), pltpu.VMEM((2, D, bt), BF16),
                            pltpu.VMEM(U.shape, BF16), pltpu.VMEM(V.shape, BF16), pltpu.VMEM(bs.shape, BF16),
                            pltpu.VMEM((L, D // 2, 128), U32), pltpu.VMEM((L, 3, R, 128), F32), pltpu.VMEM((L, 9, R, 128), F32),
                            pltpu.VMEM((ncb, D, cw), F32), pltpu.VMEM((ncb, D, cw), F32),
                            pltpu.SemaphoreType.DMA((3,)), pltpu.SemaphoreType.DMA((2,)), pltpu.SemaphoreType.DMA((2,))],
            compiler_params=pltpu.CompilerParams(vmem_limit_bytes=100*1024*1024, disable_bounds_checks=nobc),
        )(xt, U, V, bs)
        return out.T
    return fn


_FN = _make()


@jax.jit
def pallas_standalone__cross_network_dcn_v2__recsys_kernel(x0: jax.Array, U: jax.Array, V: jax.Array, bs: jax.Array):
    return _FN(x0, U, V, bs)
```

```python
import functools

import jax
import jax.numpy as jnp
from jax import lax
from jax.experimental import pallas as pl
from jax.experimental.pallas import tpu as pltpu

F32 = jnp.float32
BF16 = jnp.bfloat16
U32 = jnp.uint32

LANES = 128
NA = 6
NB = 2
LS = 2
G = 6
NG = 5
SKEW = 3
SPLIT = 2
TAIL_SPLIT = 4
NL = 9


def _kernel(x_hbm, u_hbm, v_hbm, b_hbm, o_hbm, xbuf, obuf, u_ref, v_ref, b_ref,
            uz_ref, vm_ref, vb_ref, bt_ref, x0f_ref, xf_ref, wsem, xsem, osem):
    L, D, R = u_ref.shape
    B = x_hbm.shape[1]
    first_cb = NA + NB
    body_cb = G * NG
    bt = body_cb * LANES
    f0 = first_cb * LANES
    nbody = (B - f0) // bt
    KM = (D // LANES) * LANES
    KR = D - KM
    assert f0 + nbody * bt == B and nbody >= 2
    assert KR == 32 and R + KR - 8 == LANES and L <= 8 and 0 < LS < L

    def x_copy(col0, slot):
        return pltpu.make_async_copy(x_hbm.at[:, pl.ds(col0, bt)], xbuf.at[slot], xsem.at[slot])

    def o_copy(col0, c0, n, slot):
        w = n * LANES
        return pltpu.make_async_copy(obuf.at[slot, :, pl.ds(c0 * LANES, w)],
                                     o_hbm.at[:, pl.ds(col0 + c0 * LANES, w)], osem.at[slot])

    va_cp = pltpu.make_async_copy(v_hbm.at[0:LS], v_ref.at[0:LS], wsem.at[0])
    ua_cp = pltpu.make_async_copy(u_hbm.at[0:LS], u_ref.at[0:LS], wsem.at[1])
    b_cp = pltpu.make_async_copy(b_hbm, b_ref, wsem.at[2])
    vb_cp = pltpu.make_async_copy(v_hbm.at[LS:L], v_ref.at[LS:L], wsem.at[3])
    ub_cp = pltpu.make_async_copy(u_hbm.at[LS:L], u_ref.at[LS:L], wsem.at[4])
    xa_cp = pltpu.make_async_copy(x_hbm.at[:, pl.ds(0, NA * LANES)],
                                  xbuf.at[0, :, pl.ds(0, NA * LANES)], wsem.at[5])
    xb_cp = pltpu.make_async_copy(x_hbm.at[:, pl.ds(NA * LANES, NB * LANES)],
                                  xbuf.at[0, :, pl.ds(NA * LANES, NB * LANES)], wsem.at[6])
    va_cp.start()
    b_cp.start()
    ua_cp.start()
    xa_cp.start(priority=1)

    def left_pos(l, k):
        return k if k < 8 else 8 + l

    ws = {}

    def pre_w(l):
        row = lax.broadcasted_iota(jnp.int32, (R, LANES), 0)
        col = lax.broadcasted_iota(jnp.int32, (R, LANES), 1)
        vr = v_ref[l, :, KM:D].astype(F32)
        w = jnp.concatenate([jnp.zeros((R, LANES - KR), F32), vr], axis=1)
        ws[l] = jnp.where(col < R, jnp.where(row == col, 1.0, 0.0), w).astype(BF16)

    def pre_v(l, nxlu):
        rk = lax.broadcasted_iota(jnp.int32, (KR, LANES), 0)
        for kt in range(KM // LANES):
            vm_ref[l, kt] = v_ref[l, :, kt * LANES:(kt + 1) * LANES].astype(F32)
        vr = v_ref[l, :, KM:D].astype(F32)
        for k in range(NL):
            p = left_pos(l, k)
            if k < nxlu:
                vb_ref[l, k] = jnp.broadcast_to(vr[:, p:p + 1], (R, LANES))
            else:
                vb_ref[l, k] = jnp.dot(vr, jnp.where(rk == p, 1.0, 0.0), preferred_element_type=F32)

    def pre_u(l):
        h = D // 2
        lane = lax.broadcasted_iota(jnp.int32, (h, LANES), 1)
        for r0 in (0, h):
            uz = jnp.dot(u_ref[l, r0:r0 + h, :], ws[l], preferred_element_type=F32)
            uz = jnp.where(lane == R + l, bt_ref[r0:r0 + h, :], uz)
            uz = pltpu.bitcast(uz.astype(BF16), U32)
            if r0 == 0:
                uz_ref[l, KR // 2:(KR + h) // 2, :] = uz
            else:
                uz_ref[l, (KR + h) // 2:, :] = uz[:(KM - h) // 2]
                uz_ref[l, 0:KR // 2, :] = uz[(KM - h) // 2:]

    va_cp.wait()
    b_cp.wait()
    ua_cp.wait()
    vb_cp.start(priority=1)
    ub_cp.start(priority=1)
    xb_cp.start(priority=1)
    for l in range(LS):
        pre_w(l)
    rl = lax.broadcasted_iota(jnp.int32, (L, LANES), 0)
    cl = lax.broadcasted_iota(jnp.int32, (L, LANES), 1)
    esel = jnp.where(cl == rl + R, 1.0, 0.0).astype(BF16)
    bt_ref[...] = lax.dot_general(b_ref[...], esel, (((0,), (0,)), ((), ())),
                                  preferred_element_type=F32)
    for l in range(LS):
        pre_u(l)
    for l in range(LS):
        pre_v(l, 5)

    sub = lax.broadcasted_iota(jnp.int32, (8, LANES), 0)

    def cs(c):
        return slice(c * LANES, (c + 1) * LANES)

    def compute(ticks, col0, slot, outs, ntail, hooks=None):
        x0_ref = xbuf.at[slot]
        o_ref = obuf.at[slot]
        zs = {}
        hooks = hooks or {}

        def stage_mm1(l, c, s):
            src = x0f_ref if l == 0 else xf_ref
            acc = None
            for k in range(NL):
                p = left_pos(l, k)
                t = vb_ref[l, k] * src[s, p:p + 1, :]
                acc = t if acc is None else acc + t
            for kt in range(KM // LANES):
                if l == 0:
                    xb = x0_ref[kt * LANES:(kt + 1) * LANES, cs(c)]
                else:
                    xb = xf_ref[s, KR + kt * LANES:KR + (kt + 1) * LANES, :]
                acc = acc + jnp.dot(vm_ref[l, kt], xb, preferred_element_type=F32)
            ones_row = jnp.where(sub == l, 1.0, src[s, 8:16, :])
            zs[c] = jnp.concatenate([acc, ones_row, src[s, 16:KR, :]], axis=0)

        def stage_mm2(l, c, s, nsplit):
            bounds = [((D // 16) * j // nsplit) * 16 for j in range(nsplit + 1)]
            for r0, r1 in zip(bounds[:-1], bounds[1:]):
                lhs = pltpu.bitcast(uz_ref[l, r0 // 2:r1 // 2, :], BF16)
                y = jnp.dot(lhs, zs[c], preferred_element_type=F32)
                x0 = x0f_ref[s, r0:r1, :]
                x = x0 if l == 0 else xf_ref[s, r0:r1, :]
                xn = x0 * y + x
                if l < L - 1:
                    xf_ref[s, r0:r1, :] = xn
                elif r0 == 0:
                    o_ref[KM:D, cs(c)] = xn[:KR].astype(BF16)
                    o_ref[0:r1 - KR, cs(c)] = xn[KR:].astype(BF16)
                else:
                    o_ref[r0 - KR:r1 - KR, cs(c)] = xn.astype(BF16)

        total = len(ticks)
        done = set()
        for t in range(total + SKEW):
            for h in hooks.get(t, ()):
                h()
            if t < total:
                l, c, s = ticks[t]
                assert all(ticks[q][2] != s for q in range(max(t - SKEW, 0), t))
                if l == 0:
                    x0f_ref[s, 0:KR, :] = x0_ref[KM:D, cs(c)].astype(F32)
                    x0f_ref[s, KR:D, :] = x0_ref[0:KM, cs(c)].astype(F32)
                stage_mm1(l, c, s)
            q = t - SKEW
            if q >= 0:
                l, c, s = ticks[q]
                stage_mm2(l, c, s, TAIL_SPLIT if q >= total - ntail else SPLIT)
                if l == L - 1:
                    done.add(c)
                    if c in outs:
                        c0, n = outs[c]
                        assert all(j in done for j in range(c0, c0 + n))
                        o_copy(col0, c0, n, slot).start()

    xa_cp.wait()
    x_copy(f0, 1).start(priority=1)
    compute([(l, c, c) for l in range(LS) for c in range(NA)], 0, 0, {}, 2)

    vb_cp.wait()
    ub_cp.wait()
    xb_cp.wait()
    a_ticks = [(l, c, c) for l in range(LS, L) for c in range(NA)]
    ticks = []
    for r in range(L):
        ticks += [(r, c, c) for c in range(NA, first_cb)]
        ticks += a_ticks[len(a_ticks) * r // L:len(a_ticks) * (r + 1) // L]
    first_use = {}
    for t, (l, _, _) in enumerate(ticks):
        first_use.setdefault(l, t)
    hooks = {0: [functools.partial(pre_w, l) for l in range(LS, L)] + [functools.partial(pre_v, LS, NL)],
             2: [functools.partial(pre_u, LS)]}
    assert first_use[LS] >= 2
    for l in range(LS + 1, L):
        hooks.setdefault(first_use[l] - 3, []).extend(
            [functools.partial(pre_v, l, NL), functools.partial(pre_u, l)])
    compute(ticks, 0, 0, {ticks[-1][1]: (0, first_cb)}, 3, hooks)

    body_ticks = [(l, gi * G + j, (gi % 2) * G + j) for gi in range(NG) for l in range(L) for j in range(G)]
    body_outs = {gi * G + G - 1: (gi * G, G) for gi in range(NG - 1)}
    body_outs.update({c: (c, 1) for c in range((NG - 1) * G, NG * G)})

    def body(i, carry):
        slot = (i + 1) & 1
        col0 = pl.multiple_of(f0 + i * bt, LANES)
        x_copy(col0, slot).wait()

        @pl.when(i == 1)
        def _():
            o_copy(0, 0, first_cb, slot).wait()

        @pl.when(i >= 2)
        def _():
            o_copy(0, 0, body_cb, slot).wait()

        @pl.when(i + 1 < nbody)
        def _():
            x_copy(col0 + bt, 1 - slot).start()

        compute(body_ticks, col0, slot, body_outs, 3)
        return carry

    lax.fori_loop(0, nbody, body, 0)
    o_copy(0, 0, body_cb, (nbody - 1) % 2).wait()
    o_copy(0, 0, body_cb, nbody % 2).wait()


@jax.jit
def pallas_standalone__cross_network_dcn_v2__recsys_kernel(
    x0: jax.Array,
    U: jax.Array,
    V: jax.Array,
    bs: jax.Array,
):
    B, D = x0.shape
    L, _, R = U.shape
    bt = G * NG * LANES
    nslot = max(NA + NB, 2 * G)
    out_t = pl.pallas_call(
        _kernel,
        in_specs=[pl.BlockSpec(memory_space=pl.ANY)] * 4,
        out_specs=pl.BlockSpec(memory_space=pl.ANY),
        out_shape=jax.ShapeDtypeStruct((D, B), x0.dtype),
        scratch_shapes=[
            pltpu.VMEM((2, D, bt), BF16),
            pltpu.VMEM((2, D, bt), BF16),
            pltpu.VMEM(U.shape, BF16),
            pltpu.VMEM(V.shape, BF16),
            pltpu.VMEM(bs.shape, BF16),
            pltpu.VMEM((L, D // 2, LANES), U32),
            pltpu.VMEM((L, D // LANES, R, LANES), F32),
            pltpu.VMEM((L, NL, R, LANES), F32),
            pltpu.VMEM((D, LANES), F32),
            pltpu.VMEM((nslot, D, LANES), F32),
            pltpu.VMEM((nslot, D, LANES), F32),
            pltpu.SemaphoreType.DMA((7,)),
            pltpu.SemaphoreType.DMA((2,)),
            pltpu.SemaphoreType.DMA((2,)),
        ],
        compiler_params=pltpu.CompilerParams(
            vmem_limit_bytes=100 * 1024 * 1024,
            disable_bounds_checks=True,
            disable_semaphore_checks=True,
        ),
    )(x0.T, U, V, bs)
    return out_t.T
```

```python
import functools

import jax
import jax.numpy as jnp
from jax import lax
from jax.experimental import pallas as pl
from jax.experimental.pallas import tpu as pltpu

F32 = jnp.float32
BF16 = jnp.bfloat16
U32 = jnp.uint32

LANES = 128
NA = 6
NB = 2
LS = 2
G = 6
NG = 5
SKEW = 3
SPLIT = 2
TAIL_SPLIT = 4
NTAIL = 2
NL = 9


def _kernel(x_hbm, u_hbm, v_hbm, b_hbm, o_hbm, xbuf, obuf, u_ref, v_ref, b_ref,
            uz_ref, vm_ref, vb_ref, bt_ref, x0f_ref, xf_ref, wsem, xsem, osem):
    L, D, R = u_ref.shape
    B = x_hbm.shape[1]
    first_cb = NA + NB
    body_cb = G * NG
    bt = body_cb * LANES
    f0 = first_cb * LANES
    nbody = (B - f0) // bt
    KM = (D // LANES) * LANES
    KR = D - KM
    assert f0 + nbody * bt == B and nbody >= 2
    assert KR == 32 and R + KR - 8 == LANES and L <= 8 and 0 < LS < L

    def x_copy(col0, slot):
        return pltpu.make_async_copy(x_hbm.at[:, pl.ds(col0, bt)], xbuf.at[slot], xsem.at[slot])

    def o_copy(col0, c0, n, slot):
        w = n * LANES
        return pltpu.make_async_copy(obuf.at[slot, :, pl.ds(c0 * LANES, w)],
                                     o_hbm.at[:, pl.ds(col0 + c0 * LANES, w)], osem.at[slot])

    va_cp = pltpu.make_async_copy(v_hbm.at[0:LS], v_ref.at[0:LS], wsem.at[0])
    ua_cp = pltpu.make_async_copy(u_hbm.at[0:LS], u_ref.at[0:LS], wsem.at[1])
    b_cp = pltpu.make_async_copy(b_hbm, b_ref, wsem.at[2])
    vb_cp = pltpu.make_async_copy(v_hbm.at[LS:L], v_ref.at[LS:L], wsem.at[3])
    ub_cp = pltpu.make_async_copy(u_hbm.at[LS:L], u_ref.at[LS:L], wsem.at[4])
    xa_cp = pltpu.make_async_copy(x_hbm.at[:, pl.ds(0, NA * LANES)],
                                  xbuf.at[0, :, pl.ds(0, NA * LANES)], wsem.at[5])
    xb_cp = pltpu.make_async_copy(x_hbm.at[:, pl.ds(NA * LANES, NB * LANES)],
                                  xbuf.at[0, :, pl.ds(NA * LANES, NB * LANES)], wsem.at[6])
    va_cp.start()
    b_cp.start()
    ua_cp.start()
    xa_cp.start(priority=1)

    def left_pos(l, k):
        return k if k < 8 else 8 + l

    ws = {}

    def pre_w(l):
        row = lax.broadcasted_iota(jnp.int32, (R, LANES), 0)
        col = lax.broadcasted_iota(jnp.int32, (R, LANES), 1)
        vr = v_ref[l, :, KM:D].astype(F32)
        w = jnp.concatenate([jnp.zeros((R, LANES - KR), F32), vr], axis=1)
        ws[l] = jnp.where(col < R, jnp.where(row == col, 1.0, 0.0), w).astype(BF16)

    def pre_v(l, nxlu):
        rk = lax.broadcasted_iota(jnp.int32, (KR, LANES), 0)
        for kt in range(KM // LANES):
            vm_ref[l, kt] = v_ref[l, :, kt * LANES:(kt + 1) * LANES].astype(F32)
        vr = v_ref[l, :, KM:D].astype(F32)
        for k in range(NL):
            p = left_pos(l, k)
            if k < nxlu:
                vb_ref[l, k] = jnp.broadcast_to(vr[:, p:p + 1], (R, LANES))
            else:
                vb_ref[l, k] = jnp.dot(vr, jnp.where(rk == p, 1.0, 0.0), preferred_element_type=F32)

    def pre_u(l):
        h = D // 2
        lane = lax.broadcasted_iota(jnp.int32, (h, LANES), 1)
        for r0 in (0, h):
            uz = jnp.dot(u_ref[l, r0:r0 + h, :], ws[l], preferred_element_type=F32)
            uz = jnp.where(lane == R + l, bt_ref[r0:r0 + h, :], uz)
            uz = pltpu.bitcast(uz.astype(BF16), U32)
            if r0 == 0:
                uz_ref[l, KR // 2:(KR + h) // 2, :] = uz
            else:
                uz_ref[l, (KR + h) // 2:, :] = uz[:(KM - h) // 2]
                uz_ref[l, 0:KR // 2, :] = uz[(KM - h) // 2:]

    sub = lax.broadcasted_iota(jnp.int32, (8, LANES), 0)

    def cs(c):
        return slice(c * LANES, (c + 1) * LANES)

    def compute(ticks, col0, slot, outs, ntail, hooks=None):
        x0_ref = xbuf.at[slot]
        o_ref = obuf.at[slot]
        zs = {}
        hooks = hooks or {}

        def stage_mm1(l, c, s):
            src = x0f_ref if l == 0 else xf_ref
            acc = None
            for k in range(NL):
                p = left_pos(l, k)
                t = vb_ref[l, k] * src[s, p:p + 1, :]
                acc = t if acc is None else acc + t
            for kt in range(KM // LANES):
                if l == 0:
                    xb = x0_ref[kt * LANES:(kt + 1) * LANES, cs(c)]
                else:
                    xb = xf_ref[s, KR + kt * LANES:KR + (kt + 1) * LANES, :]
                acc = acc + jnp.dot(vm_ref[l, kt], xb, preferred_element_type=F32)
            ones_row = jnp.where(sub == l, 1.0, src[s, 8:16, :])
            zs[c] = jnp.concatenate([acc, ones_row, src[s, 16:KR, :]], axis=0)

        def stage_mm2(l, c, s, nsplit):
            bounds = [((D // 16) * j // nsplit) * 16 for j in range(nsplit + 1)]
            for r0, r1 in zip(bounds[:-1], bounds[1:]):
                lhs = pltpu.bitcast(uz_ref[l, r0 // 2:r1 // 2, :], BF16)
                y = jnp.dot(lhs, zs[c], preferred_element_type=F32)
                x0 = x0f_ref[s, r0:r1, :]
                x = x0 if l == 0 else xf_ref[s, r0:r1, :]
                xn = x0 * y + x
                if l < L - 1:
                    xf_ref[s, r0:r1, :] = xn
                elif r0 == 0:
                    o_ref[KM:D, cs(c)] = xn[:KR].astype(BF16)
                    o_ref[0:r1 - KR, cs(c)] = xn[KR:].astype(BF16)
                else:
                    o_ref[r0 - KR:r1 - KR, cs(c)] = xn.astype(BF16)

        total = len(ticks)
        done = set()
        for t in range(total + SKEW):
            for h in hooks.get(t, ()):
                h()
            if t < total:
                l, c, s = ticks[t]
                assert all(ticks[q][2] != s for q in range(max(t - SKEW, 0), t))
                if l == 0:
                    x0f_ref[s, 0:KR, :] = x0_ref[KM:D, cs(c)].astype(F32)
                    x0f_ref[s, KR:D, :] = x0_ref[0:KM, cs(c)].astype(F32)
                stage_mm1(l, c, s)
            q = t - SKEW
            if q >= 0:
                l, c, s = ticks[q]
                stage_mm2(l, c, s, TAIL_SPLIT if q >= total - ntail else SPLIT)
                if l == L - 1:
                    done.add(c)
                    if c in outs:
                        c0, n = outs[c]
                        assert all(j in done for j in range(c0, c0 + n))
                        o_copy(col0, c0, n, slot).start()

    def first_section():
        va_cp.wait()
        b_cp.wait()
        ua_cp.wait()
        vb_cp.start(priority=1)
        ub_cp.start(priority=1)
        xb_cp.start(priority=1)
        for l in range(LS):
            pre_w(l)
        rl = lax.broadcasted_iota(jnp.int32, (L, LANES), 0)
        cl = lax.broadcasted_iota(jnp.int32, (L, LANES), 1)
        esel = jnp.where(cl == rl + R, 1.0, 0.0).astype(BF16)
        bt_ref[...] = lax.dot_general(b_ref[...], esel, (((0,), (0,)), ((), ())),
                                      preferred_element_type=F32)
        for l in range(LS):
            pre_u(l)
        for l in range(LS):
            pre_v(l, 5)

        xa_cp.wait()
        x_copy(f0, 1).start(priority=1)
        compute([(l, c, c) for l in range(LS) for c in range(NA)], 0, 0, {}, NTAIL)

        vb_cp.wait()
        ub_cp.wait()
        xb_cp.wait()
        a_ticks = [(l, c, c) for l in range(LS, L) for c in range(NA)]
        ticks = []
        for r in range(L):
            ticks += [(r, c, c) for c in range(NA, first_cb)]
            ticks += a_ticks[len(a_ticks) * r // L:len(a_ticks) * (r + 1) // L]
        first_use = {}
        for t, (l, _, _) in enumerate(ticks):
            first_use.setdefault(l, t)
        hooks = {0: [functools.partial(pre_w, l) for l in range(LS, L)] + [functools.partial(pre_v, LS, NL)],
                 2: [functools.partial(pre_u, LS)]}
        assert first_use[LS] >= 2
        for l in range(LS + 1, L):
            hooks.setdefault(first_use[l] - 5, []).extend(
                [functools.partial(pre_v, l, NL), functools.partial(pre_u, l)])
        compute(ticks, 0, 0, {ticks[-1][1]: (0, first_cb)}, NTAIL, hooks)


    body_ticks = [(l, gi * G + j, (gi % 2) * G + j) for gi in range(NG) for l in range(L) for j in range(G)]
    body_outs = {gi * G + G - 1: (gi * G, G) for gi in range(NG - 1)}
    body_outs.update({c: (c, 1) for c in range((NG - 1) * G, NG * G)})

    def body(i, carry):
        pl.when(i == 0)(first_section)
        slot = (i + 1) & 1
        col0 = pl.multiple_of(f0 + i * bt, LANES)
        x_copy(col0, slot).wait()

        @pl.when(i == 1)
        def _():
            o_copy(0, 0, first_cb, slot).wait()

        @pl.when(i >= 2)
        def _():
            o_copy(0, 0, body_cb, slot).wait()

        @pl.when(i + 1 < nbody)
        def _():
            x_copy(col0 + bt, 1 - slot).start()

        compute(body_ticks, col0, slot, body_outs, NTAIL)
        return carry

    lax.fori_loop(0, nbody, body, 0)
    o_copy(0, 0, body_cb, (nbody - 1) % 2).wait()
    o_copy(0, 0, body_cb, nbody % 2).wait()


@jax.jit
def pallas_standalone__cross_network_dcn_v2__recsys_kernel(
    x0: jax.Array,
    U: jax.Array,
    V: jax.Array,
    bs: jax.Array,
):
    B, D = x0.shape
    L, _, R = U.shape
    bt = G * NG * LANES
    nslot = max(NA + NB, 2 * G)
    out_t = pl.pallas_call(
        _kernel,
        in_specs=[pl.BlockSpec(memory_space=pl.ANY)] * 4,
        out_specs=pl.BlockSpec(memory_space=pl.ANY),
        out_shape=jax.ShapeDtypeStruct((D, B), x0.dtype),
        scratch_shapes=[
            pltpu.VMEM((2, D, bt), BF16),
            pltpu.VMEM((2, D, bt), BF16),
            pltpu.VMEM(U.shape, BF16),
            pltpu.VMEM(V.shape, BF16),
            pltpu.VMEM(bs.shape, BF16),
            pltpu.VMEM((L, D // 2, LANES), U32),
            pltpu.VMEM((L, D // LANES, R, LANES), F32),
            pltpu.VMEM((L, NL, R, LANES), F32),
            pltpu.VMEM((D, LANES), F32),
            pltpu.VMEM((nslot, D, LANES), F32),
            pltpu.VMEM((nslot, D, LANES), F32),
            pltpu.SemaphoreType.DMA((7,)),
            pltpu.SemaphoreType.DMA((2,)),
            pltpu.SemaphoreType.DMA((2,)),
        ],
        compiler_params=pltpu.CompilerParams(
            vmem_limit_bytes=100 * 1024 * 1024,
            disable_bounds_checks=True,
            disable_semaphore_checks=True,
        ),
    )(x0.T, U, V, bs)
    return out_t.T
```

```python
import functools

import jax
import jax.numpy as jnp
from jax import lax
from jax.experimental import pallas as pl
from jax.experimental.pallas import tpu as pltpu

F32 = jnp.float32
BF16 = jnp.bfloat16
U32 = jnp.uint32

LANES = 128
NA = 6
NB = 2
LS = 2
G = 6
NG = 5
SKEW = 3
SPLIT = 2
TAIL_SPLIT = 4
NL = 9

_dot = functools.partial(jnp.dot, preferred_element_type=F32, precision=lax.Precision.DEFAULT)


def _kernel(x_hbm, u_hbm, v_hbm, b_hbm, o_hbm, xbuf, obuf, u_ref, v_ref, b_ref,
            uz_ref, vm_ref, vb_ref, x0f_ref, xf_ref, wsem, xsem, osem):
    L, D, R = u_ref.shape
    B = x_hbm.shape[1]
    first_cb = NA + NB
    body_cb = G * NG
    bt = body_cb * LANES
    f0 = first_cb * LANES
    nbody = (B - f0) // bt
    KM = (D // LANES) * LANES
    KR = D - KM
    assert f0 + nbody * bt == B and nbody >= 2
    assert KR == 32 and R + KR - 8 == LANES and L <= 8 and 0 < LS < L

    def x_copy(col0, slot):
        return pltpu.make_async_copy(x_hbm.at[:, pl.ds(col0, bt)], xbuf.at[slot], xsem.at[slot])

    def o_copy(col0, c0, n, slot):
        w = n * LANES
        return pltpu.make_async_copy(obuf.at[slot, :, pl.ds(c0 * LANES, w)],
                                     o_hbm.at[:, pl.ds(col0 + c0 * LANES, w)], osem.at[slot])

    cols_a = pl.ds(0, NA * LANES)
    cols_b = pl.ds(NA * LANES, NB * LANES)
    va_cp = pltpu.make_async_copy(v_hbm.at[0:LS], v_ref.at[0:LS], wsem.at[0])
    ua_cp = pltpu.make_async_copy(u_hbm.at[0:LS], u_ref.at[0:LS], wsem.at[1])
    xa_cp = pltpu.make_async_copy(x_hbm.at[:, cols_a], xbuf.at[0, :, cols_a], wsem.at[2])
    vb_cp = pltpu.make_async_copy(v_hbm.at[LS:L], v_ref.at[LS:L], wsem.at[3])
    ub_cp = pltpu.make_async_copy(u_hbm.at[LS:L], u_ref.at[LS:L], wsem.at[4])
    xb_cp = pltpu.make_async_copy(x_hbm.at[:, cols_b], xbuf.at[0, :, cols_b], wsem.at[5])
    b_cp = pltpu.make_async_copy(b_hbm, b_ref, wsem.at[6])
    va_cp.start()
    ua_cp.start()
    b_cp.start()
    xa_cp.start(priority=1)

    def left_pos(l, k):
        return k if k < 8 else 8 + l

    def pre_v(l, nxlu):
        rk = lax.broadcasted_iota(jnp.int32, (KR, LANES), 0)
        for kt in range(KM // LANES):
            vm_ref[l, kt] = v_ref[l, :, kt * LANES:(kt + 1) * LANES].astype(F32)
        vr = v_ref[l, :, KM:D].astype(F32)
        for k in range(NL):
            p = left_pos(l, k)
            if k < nxlu:
                vb_ref[l, k] = jnp.broadcast_to(vr[:, p:p + 1], (R, LANES))
            else:
                vb_ref[l, k] = _dot(vr, jnp.where(rk == p, 1.0, 0.0))

    def pre_u(l):
        vzt = v_ref[l, :, KM:D].astype(F32).T[8:]
        pt = lax.dot_general(vzt, u_ref[l], (((1,), (1,)), ((), ())), preferred_element_type=F32,
                             precision=lax.Precision.DEFAULT)
        rowi = lax.broadcasted_iota(jnp.int32, (8, D), 0)
        top = jnp.where(rowi == l, b_ref[l:l + 1, :].astype(F32), pt[:8])
        p = jnp.concatenate([jnp.zeros((R, D), F32), top, pt[8:]], axis=0).T
        uz = jnp.concatenate([u_ref[l].astype(F32), p[:, R:]], axis=1)
        uz = pltpu.bitcast(uz.astype(BF16), U32)
        uz_ref[l, KR // 2:, :] = uz[:KM // 2]
        uz_ref[l, 0:KR // 2, :] = uz[KM // 2:]

    sub = lax.broadcasted_iota(jnp.int32, (8, LANES), 0)

    def cs(c):
        return slice(c * LANES, (c + 1) * LANES)

    def compute(ticks, col0, slot, outs, ntail, hooks=None):
        x0_ref = xbuf.at[slot]
        o_ref = obuf.at[slot]
        zs = {}
        hooks = hooks or {}

        def stage_mm1(l, c, s):
            src = x0f_ref if l == 0 else xf_ref
            acc = None
            for k in range(NL):
                p = left_pos(l, k)
                t = vb_ref[l, k] * src[s, p:p + 1, :]
                acc = t if acc is None else acc + t
            for kt in range(KM // LANES):
                if l == 0:
                    xb = x0_ref[kt * LANES:(kt + 1) * LANES, cs(c)]
                else:
                    xb = xf_ref[s, KR + kt * LANES:KR + (kt + 1) * LANES, :]
                acc = acc + _dot(vm_ref[l, kt], xb)
            ones_row = jnp.where(sub == l, 1.0, src[s, 8:16, :])
            zs[c] = jnp.concatenate([acc, ones_row, src[s, 16:KR, :]], axis=0)

        def stage_mm2(l, c, s, nsplit):
            bounds = [((D // 16) * j // nsplit) * 16 for j in range(nsplit + 1)]
            for r0, r1 in zip(bounds[:-1], bounds[1:]):
                y = _dot(pltpu.bitcast(uz_ref[l, r0 // 2:r1 // 2, :], BF16), zs[c])
                x0 = x0f_ref[s, r0:r1, :]
                x = x0 if l == 0 else xf_ref[s, r0:r1, :]
                xn = x0 * y + x
                if l < L - 1:
                    xf_ref[s, r0:r1, :] = xn
                elif r0 == 0:
                    o_ref[KM:D, cs(c)] = xn[:KR].astype(BF16)
                    o_ref[0:r1 - KR, cs(c)] = xn[KR:].astype(BF16)
                else:
                    o_ref[r0 - KR:r1 - KR, cs(c)] = xn.astype(BF16)

        total = len(ticks)
        done = set()
        for t in range(total + SKEW):
            for h in hooks.get(t, ()):
                h()
            if t < total:
                l, c, s = ticks[t]
                assert all(ticks[q][2] != s for q in range(max(t - SKEW, 0), t))
                if l == 0:
                    x0f_ref[s, 0:KR, :] = x0_ref[KM:D, cs(c)].astype(F32)
                    x0f_ref[s, KR:D, :] = x0_ref[0:KM, cs(c)].astype(F32)
                stage_mm1(l, c, s)
            q = t - SKEW
            if q >= 0:
                l, c, s = ticks[q]
                stage_mm2(l, c, s, TAIL_SPLIT if q >= total - ntail else SPLIT)
                if l == L - 1:
                    done.add(c)
                    if c in outs:
                        c0, n = outs[c]
                        assert all(j in done for j in range(c0, c0 + n))
                        o_copy(col0, c0, n, slot).start()

    def first_section():
        va_cp.wait()
        ua_cp.wait()
        b_cp.wait()
        vb_cp.start(priority=1)
        ub_cp.start(priority=1)
        xb_cp.start(priority=1)
        for l in range(LS):
            pre_v(l, 5)
        for l in range(LS):
            pre_u(l)

        xa_cp.wait()
        x_copy(f0, 1).start(priority=1)
        compute([(l, c, c) for l in range(LS) for c in range(NA)], 0, 0, {}, 2)

        vb_cp.wait()
        ub_cp.wait()
        xb_cp.wait()
        a_ticks = [(l, c, c) for l in range(LS, L) for c in range(NA)]
        ticks = []
        for r in range(L):
            ticks += [(r, c, c) for c in range(NA, first_cb)]
            ticks += a_ticks[len(a_ticks) * r // L:len(a_ticks) * (r + 1) // L]
        first_use = {}
        for t, (l, _, _) in enumerate(ticks):
            first_use.setdefault(l, t)
        hooks = {0: [functools.partial(pre_v, l, NL) for l in range(LS, L)]}
        for l in range(LS, L):
            pos = 3 if l == LS else first_use[l] - 3
            assert 0 <= pos <= first_use[l] + SKEW
            hooks.setdefault(pos, []).append(functools.partial(pre_u, l))
        compute(ticks, 0, 0, {ticks[-1][1]: (0, first_cb)}, 3, hooks)

    body_ticks = [(l, gi * G + j, (gi % 2) * G + j) for gi in range(NG) for l in range(L) for j in range(G)]
    body_outs = {gi * G + G - 1: (gi * G, G) for gi in range(NG - 1)}
    body_outs.update({c: (c, 1) for c in range((NG - 1) * G, NG * G)})

    def body(i, carry):
        pl.when(i == 0)(first_section)
        slot = (i + 1) & 1
        col0 = pl.multiple_of(f0 + i * bt, LANES)
        x_copy(col0, slot).wait()

        @pl.when(i == 1)
        def _():
            o_copy(0, 0, first_cb, slot).wait()

        @pl.when(i >= 2)
        def _():
            o_copy(0, 0, body_cb, slot).wait()

        @pl.when(i + 1 < nbody)
        def _():
            x_copy(col0 + bt, 1 - slot).start()

        compute(body_ticks, col0, slot, body_outs, 2)
        return carry

    lax.fori_loop(0, nbody, body, 0)
    o_copy(0, 0, body_cb, (nbody - 1) % 2).wait()
    o_copy(0, 0, body_cb, nbody % 2).wait()


@jax.jit
def pallas_standalone__cross_network_dcn_v2__recsys_kernel(
    x0: jax.Array,
    U: jax.Array,
    V: jax.Array,
    bs: jax.Array,
):
    B, D = x0.shape
    L, _, R = U.shape
    bt = G * NG * LANES
    nslot = max(NA + NB, 2 * G)
    out_t = pl.pallas_call(
        _kernel,
        in_specs=[pl.BlockSpec(memory_space=pl.ANY)] * 4,
        out_specs=pl.BlockSpec(memory_space=pl.ANY),
        out_shape=jax.ShapeDtypeStruct((D, B), x0.dtype),
        scratch_shapes=[
            pltpu.VMEM((2, D, bt), BF16),
            pltpu.VMEM((2, D, bt), BF16),
            pltpu.VMEM(U.shape, BF16),
            pltpu.VMEM(V.shape, BF16),
            pltpu.VMEM(bs.shape, BF16),
            pltpu.VMEM((L, D // 2, LANES), U32),
            pltpu.VMEM((L, D // LANES, R, LANES), F32),
            pltpu.VMEM((L, NL, R, LANES), F32),
            pltpu.VMEM((nslot, D, LANES), F32),
            pltpu.VMEM((nslot, D, LANES), F32),
            pltpu.SemaphoreType.DMA((7,)),
            pltpu.SemaphoreType.DMA((2,)),
            pltpu.SemaphoreType.DMA((2,)),
        ],
        compiler_params=pltpu.CompilerParams(
            vmem_limit_bytes=64 * 1024 * 1024,
            disable_bounds_checks=True,
            disable_semaphore_checks=True,
        ),
    )(x0.T, U, V, bs)
    return out_t.T
```

```python
import functools

import jax
import jax.numpy as jnp
from jax import lax
from jax.experimental import pallas as pl
from jax.experimental.pallas import tpu as pltpu

F32 = jnp.float32
BF16 = jnp.bfloat16
U32 = jnp.uint32

LANES = 128
NA = 6
NB = 2
LS = 2
G = 5
NG = 6
SPLIT = 2
TAIL_SPLIT = 4
NL = 9

_dot = functools.partial(jnp.dot, preferred_element_type=F32, precision=lax.Precision.DEFAULT)


def _kernel(x_hbm, u_hbm, v_hbm, b_hbm, o_hbm, xbuf, obuf, u_ref, v_ref, b_ref,
            uz_ref, vm_ref, vb_ref, x0f_ref, xf_ref, wsem, xsem, osem):
    L, D, R = u_ref.shape
    B = x_hbm.shape[1]
    first_cb = NA + NB
    body_cb = G * NG
    bt = body_cb * LANES
    f0 = first_cb * LANES
    nbody = (B - f0) // bt
    KM = (D // LANES) * LANES
    KR = D - KM
    assert f0 + nbody * bt == B and nbody >= 2
    assert KR == 32 and R + KR - 8 == LANES and L <= 8 and 0 < LS < L

    def x_copy(col0, slot):
        return pltpu.make_async_copy(x_hbm.at[:, pl.ds(col0, bt)], xbuf.at[slot], xsem.at[slot])

    def o_copy(col0, c0, n, slot):
        w = n * LANES
        return pltpu.make_async_copy(obuf.at[slot, :, pl.ds(c0 * LANES, w)],
                                     o_hbm.at[:, pl.ds(col0 + c0 * LANES, w)], osem.at[slot])

    cols_a = pl.ds(0, NA * LANES)
    cols_b = pl.ds(NA * LANES, NB * LANES)
    va_cp = pltpu.make_async_copy(v_hbm.at[0:LS], v_ref.at[0:LS], wsem.at[0])
    ua_cp = pltpu.make_async_copy(u_hbm.at[0:LS], u_ref.at[0:LS], wsem.at[1])
    xa_cp = pltpu.make_async_copy(x_hbm.at[:, cols_a], xbuf.at[0, :, cols_a], wsem.at[2])
    vb_cp = pltpu.make_async_copy(v_hbm.at[LS:L], v_ref.at[LS:L], wsem.at[3])
    ub_cp = pltpu.make_async_copy(u_hbm.at[LS:L], u_ref.at[LS:L], wsem.at[4])
    xb_cp = pltpu.make_async_copy(x_hbm.at[:, cols_b], xbuf.at[0, :, cols_b], wsem.at[5])
    b_cp = pltpu.make_async_copy(b_hbm, b_ref, wsem.at[6])
    va_cp.start()
    ua_cp.start()
    b_cp.start()
    xa_cp.start(priority=1)

    def left_pos(l, k):
        return k if k < 8 else 8 + l

    def pre_v(l, nxlu):
        rk = lax.broadcasted_iota(jnp.int32, (KR, LANES), 0)
        for kt in range(KM // LANES):
            vm_ref[l, kt] = v_ref[l, :, kt * LANES:(kt + 1) * LANES].astype(F32)
        vr = v_ref[l, :, KM:D].astype(F32)
        for k in range(NL):
            p = left_pos(l, k)
            if k < nxlu:
                vb_ref[l, k] = jnp.broadcast_to(vr[:, p:p + 1], (R, LANES))
            else:
                vb_ref[l, k] = _dot(vr, jnp.where(rk == p, 1.0, 0.0))

    def pre_u(l):
        vzt = v_ref[l, :, KM:D].astype(F32).T[8:]
        pt = lax.dot_general(vzt, u_ref[l], (((1,), (1,)), ((), ())), preferred_element_type=F32,
                             precision=lax.Precision.DEFAULT)
        rowi = lax.broadcasted_iota(jnp.int32, (8, D), 0)
        top = jnp.where(rowi == l, b_ref[l:l + 1, :].astype(F32), pt[:8])
        p = jnp.concatenate([jnp.zeros((R, D), F32), top, pt[8:]], axis=0).T
        uz = jnp.concatenate([u_ref[l].astype(F32), p[:, R:]], axis=1)
        uz = pltpu.bitcast(uz.astype(BF16), U32)
        uz_ref[l, KR // 2:, :] = uz[:KM // 2]
        uz_ref[l, 0:KR // 2, :] = uz[KM // 2:]

    sub = lax.broadcasted_iota(jnp.int32, (8, LANES), 0)

    def cs(c):
        return slice(c * LANES, (c + 1) * LANES)

    def compute(ticks, col0, slot, outs, skew, ntail, hooks=None):
        x0_ref = xbuf.at[slot]
        o_ref = obuf.at[slot]
        zs = {}
        hooks = hooks or {}

        def stage_mm1(l, c, s):
            src = x0f_ref if l == 0 else xf_ref
            acc = None
            for k in range(NL):
                p = left_pos(l, k)
                t = vb_ref[l, k] * src[s, p:p + 1, :]
                acc = t if acc is None else acc + t
            for kt in range(KM // LANES):
                if l == 0:
                    xb = x0_ref[kt * LANES:(kt + 1) * LANES, cs(c)]
                else:
                    xb = xf_ref[s, KR + kt * LANES:KR + (kt + 1) * LANES, :]
                acc = acc + _dot(vm_ref[l, kt], xb)
            ones_row = jnp.where(sub == l, 1.0, src[s, 8:16, :])
            zs[c] = jnp.concatenate([acc, ones_row, src[s, 16:KR, :]], axis=0)

        def stage_mm2(l, c, s, nsplit):
            bounds = [((D // 16) * j // nsplit) * 16 for j in range(nsplit + 1)]
            for r0, r1 in zip(bounds[:-1], bounds[1:]):
                y = _dot(pltpu.bitcast(uz_ref[l, r0 // 2:r1 // 2, :], BF16), zs[c])
                x0 = x0f_ref[s, r0:r1, :]
                x = x0 if l == 0 else xf_ref[s, r0:r1, :]
                xn = x0 * y + x
                if l < L - 1:
                    xf_ref[s, r0:r1, :] = xn
                elif r0 == 0:
                    o_ref[KM:D, cs(c)] = xn[:KR].astype(BF16)
                    o_ref[0:r1 - KR, cs(c)] = xn[KR:].astype(BF16)
                else:
                    o_ref[r0 - KR:r1 - KR, cs(c)] = xn.astype(BF16)

        total = len(ticks)
        done = set()
        for t in range(total + skew):
            for h in hooks.get(t, ()):
                h()
            if t < total:
                l, c, s = ticks[t]
                assert all(ticks[q][2] != s for q in range(max(t - skew, 0), t))
                if l == 0:
                    x0f_ref[s, 0:KR, :] = x0_ref[KM:D, cs(c)].astype(F32)
                    x0f_ref[s, KR:D, :] = x0_ref[0:KM, cs(c)].astype(F32)
                stage_mm1(l, c, s)
            q = t - skew
            if q >= 0:
                l, c, s = ticks[q]
                stage_mm2(l, c, s, TAIL_SPLIT if q >= total - ntail else SPLIT)
                if l == L - 1:
                    done.add(c)
                    if c in outs:
                        c0, n = outs[c]
                        assert all(j in done for j in range(c0, c0 + n))
                        o_copy(col0, c0, n, slot).start()

    def first_section():
        va_cp.wait()
        ua_cp.wait()
        b_cp.wait()
        vb_cp.start(priority=1)
        ub_cp.start(priority=1)
        xb_cp.start(priority=1)
        for l in range(LS):
            pre_v(l, 5)
        for l in range(LS):
            pre_u(l)

        xa_cp.wait()
        x_copy(f0, 1).start(priority=1)
        compute([(l, c, c) for l in range(LS) for c in range(NA)], 0, 0, {}, 3, 2)

        vb_cp.wait()
        ub_cp.wait()
        xb_cp.wait()
        a_ticks = [(l, c, c) for l in range(LS, L) for c in range(NA)]
        ticks = []
        for r in range(L):
            ticks += [(r, c, c) for c in range(NA, first_cb)]
            ticks += a_ticks[len(a_ticks) * r // L:len(a_ticks) * (r + 1) // L]
        first_use = {}
        for t, (l, _, _) in enumerate(ticks):
            first_use.setdefault(l, t)
        hooks = {0: [functools.partial(pre_v, l, NL) for l in range(LS, L)]}
        for l in range(LS, L):
            pos = 3 if l == LS else first_use[l] - 3
            assert 0 <= pos <= first_use[l] + 3
            hooks.setdefault(pos, []).append(functools.partial(pre_u, l))
        compute(ticks, 0, 0, {ticks[-1][1]: (0, first_cb)}, 3, 3, hooks)

    body_ticks = [(l, gi * G + j, (gi % 2) * G + j) for gi in range(NG) for l in range(L) for j in range(G)]
    body_outs = {gi * G + G - 1: (gi * G, G) for gi in range(NG - 1)}
    body_outs.update({c: (c, 1) for c in range((NG - 1) * G, NG * G)})

    def body(i, carry):
        pl.when(i == 0)(first_section)
        slot = (i + 1) & 1
        col0 = pl.multiple_of(f0 + i * bt, LANES)
        x_copy(col0, slot).wait()

        @pl.when(i == 1)
        def _():
            o_copy(0, 0, first_cb, slot).wait()

        @pl.when(i >= 2)
        def _():
            o_copy(0, 0, body_cb, slot).wait()

        @pl.when(i + 1 < nbody)
        def _():
            x_copy(col0 + bt, 1 - slot).start()

        compute(body_ticks, col0, slot, body_outs, 2, 3)
        return carry

    lax.fori_loop(0, nbody, body, 0)
    o_copy(0, 0, body_cb, (nbody - 1) % 2).wait()
    o_copy(0, 0, body_cb, nbody % 2).wait()


@jax.jit
def pallas_standalone__cross_network_dcn_v2__recsys_kernel(
    x0: jax.Array,
    U: jax.Array,
    V: jax.Array,
    bs: jax.Array,
):
    B, D = x0.shape
    L, _, R = U.shape
    bt = G * NG * LANES
    nslot = max(NA + NB, 2 * G)
    out_t = pl.pallas_call(
        _kernel,
        in_specs=[pl.BlockSpec(memory_space=pl.ANY)] * 4,
        out_specs=pl.BlockSpec(memory_space=pl.ANY),
        out_shape=jax.ShapeDtypeStruct((D, B), x0.dtype),
        scratch_shapes=[
            pltpu.VMEM((2, D, bt), BF16),
            pltpu.VMEM((2, D, bt), BF16),
            pltpu.VMEM(U.shape, BF16),
            pltpu.VMEM(V.shape, BF16),
            pltpu.VMEM(bs.shape, BF16),
            pltpu.VMEM((L, D // 2, LANES), U32),
            pltpu.VMEM((L, D // LANES, R, LANES), F32),
            pltpu.VMEM((L, NL, R, LANES), F32),
            pltpu.VMEM((nslot, D, LANES), F32),
            pltpu.VMEM((nslot, D, LANES), F32),
            pltpu.SemaphoreType.DMA((7,)),
            pltpu.SemaphoreType.DMA((2,)),
            pltpu.SemaphoreType.DMA((2,)),
        ],
        compiler_params=pltpu.CompilerParams(
            vmem_limit_bytes=64 * 1024 * 1024,
            disable_bounds_checks=True,
            disable_semaphore_checks=True,
        ),
    )(x0.T, U, V, bs)
    return out_t.T
```

```python
import functools

import jax
import jax.numpy as jnp
from jax import lax
from jax.experimental import pallas as pl
from jax.experimental.pallas import tpu as pltpu

F32 = jnp.float32
BF16 = jnp.bfloat16

LANES = 128
NA = 6
NB = 2
LS = 2
G = 5
NG = 6
SPLIT = 2
TAIL_SPLIT = 4
NL = 9

_dot = functools.partial(jnp.dot, preferred_element_type=F32, precision=lax.Precision.DEFAULT)


def _kernel(x_hbm, u_hbm, v_hbm, b_hbm, o_hbm, xbuf, obuf, u_ref, v_ref, b_ref,
            uz_ref, vm_ref, vb_ref, x0f_ref, xf_ref, wsem, xsem, osem):
    L, D, R = u_ref.shape
    B = x_hbm.shape[1]
    first_cb = NA + NB
    body_cb = G * NG
    bt = body_cb * LANES
    f0 = first_cb * LANES
    nbody = (B - f0) // bt
    KM = (D // LANES) * LANES
    KR = D - KM
    assert f0 + nbody * bt == B and nbody >= 2
    assert KR == 32 and R + KR - 8 == LANES and L <= 8 and 0 < LS < L

    def x_copy(col0, slot):
        return pltpu.make_async_copy(x_hbm.at[:, pl.ds(col0, bt)], xbuf.at[slot], xsem.at[slot])

    def o_copy(col0, c0, n, slot):
        w = n * LANES
        return pltpu.make_async_copy(obuf.at[slot, :, pl.ds(c0 * LANES, w)],
                                     o_hbm.at[:, pl.ds(col0 + c0 * LANES, w)], osem.at[slot])

    cols_a = pl.ds(0, NA * LANES)
    cols_b = pl.ds(NA * LANES, NB * LANES)
    va_cp = pltpu.make_async_copy(v_hbm.at[0:LS], v_ref.at[0:LS], wsem.at[0])
    ua_cp = pltpu.make_async_copy(u_hbm.at[0:LS], u_ref.at[0:LS], wsem.at[1])
    xa_cp = pltpu.make_async_copy(x_hbm.at[:, cols_a], xbuf.at[0, :, cols_a], wsem.at[2])
    vb_cp = pltpu.make_async_copy(v_hbm.at[LS:L], v_ref.at[LS:L], wsem.at[3])
    ub_cp = pltpu.make_async_copy(u_hbm.at[LS:L], u_ref.at[LS:L], wsem.at[4])
    xb_cp = pltpu.make_async_copy(x_hbm.at[:, cols_b], xbuf.at[0, :, cols_b], wsem.at[5])
    b_cp = pltpu.make_async_copy(b_hbm, b_ref, wsem.at[6])
    va_cp.start()
    ua_cp.start()
    b_cp.start()
    xa_cp.start(priority=1)

    def left_pos(l, k):
        return k if k < 8 else 8 + l

    def pre_v(l, nxlu):
        rk = lax.broadcasted_iota(jnp.int32, (KR, LANES), 0)
        for kt in range(KM // LANES):
            vm_ref[l, kt] = v_ref[l, :, kt * LANES:(kt + 1) * LANES].astype(F32)
        vr = v_ref[l, :, KM:D].astype(F32)
        for k in range(NL):
            p = left_pos(l, k)
            if k < nxlu:
                vb_ref[l, k] = jnp.broadcast_to(vr[:, p:p + 1], (R, LANES))
            else:
                vb_ref[l, k] = _dot(vr, jnp.where(rk == p, 1.0, 0.0))

    def pre_u(l):
        vzt = v_ref[l, :, KM:D].astype(F32).T[8:]
        pt = lax.dot_general(vzt, u_ref[l], (((1,), (1,)), ((), ())), preferred_element_type=F32,
                             precision=lax.Precision.DEFAULT)
        rowi = lax.broadcasted_iota(jnp.int32, (8, D), 0)
        top = jnp.where(rowi == l, b_ref[l:l + 1, :].astype(F32), pt[:8])
        p = jnp.concatenate([jnp.zeros((R, D), F32), top, pt[8:]], axis=0).T
        uz = jnp.concatenate([u_ref[l].astype(F32), p[:, R:]], axis=1)
        uz_ref[l, KR:, :] = uz[:KM].astype(BF16)
        uz_ref[l, 0:KR, :] = uz[KM:].astype(BF16)

    sub = lax.broadcasted_iota(jnp.int32, (8, LANES), 0)

    def cs(c):
        return slice(c * LANES, (c + 1) * LANES)

    def compute(ticks, col0, slot, outs, skew, ntail, hooks=None):
        x0_ref = xbuf.at[slot]
        o_ref = obuf.at[slot]
        zs = {}
        hooks = hooks or {}

        def stage_mm1(l, c, s):
            src = x0f_ref if l == 0 else xf_ref
            acc = None
            for k in range(NL):
                p = left_pos(l, k)
                t = vb_ref[l, k] * src[s, p:p + 1, :]
                acc = t if acc is None else acc + t
            for kt in range(KM // LANES):
                if l == 0:
                    xb = x0_ref[kt * LANES:(kt + 1) * LANES, cs(c)]
                else:
                    xb = xf_ref[s, KR + kt * LANES:KR + (kt + 1) * LANES, :]
                acc = acc + _dot(vm_ref[l, kt], xb)
            ones_row = jnp.where(sub == l, 1.0, src[s, 8:16, :])
            zs[c] = jnp.concatenate([acc, ones_row, src[s, 16:KR, :]], axis=0)

        def stage_mm2(l, c, s, nsplit):
            bounds = [((D // 16) * j // nsplit) * 16 for j in range(nsplit + 1)]
            for r0, r1 in zip(bounds[:-1], bounds[1:]):
                y = _dot(uz_ref[l, r0:r1, :], zs[c])
                x0 = x0f_ref[s, r0:r1, :]
                x = x0 if l == 0 else xf_ref[s, r0:r1, :]
                xn = x0 * y + x
                if l < L - 1:
                    xf_ref[s, r0:r1, :] = xn
                elif r0 == 0:
                    o_ref[KM:D, cs(c)] = xn[:KR].astype(BF16)
                    o_ref[0:r1 - KR, cs(c)] = xn[KR:].astype(BF16)
                else:
                    o_ref[r0 - KR:r1 - KR, cs(c)] = xn.astype(BF16)

        total = len(ticks)
        done = set()
        for t in range(total + skew):
            for h in hooks.get(t, ()):
                h()
            if t < total:
                l, c, s = ticks[t]
                assert all(ticks[q][2] != s for q in range(max(t - skew, 0), t))
                if l == 0:
                    x0f_ref[s, 0:KR, :] = x0_ref[KM:D, cs(c)].astype(F32)
                    x0f_ref[s, KR:D, :] = x0_ref[0:KM, cs(c)].astype(F32)
                stage_mm1(l, c, s)
            q = t - skew
            if q >= 0:
                l, c, s = ticks[q]
                stage_mm2(l, c, s, TAIL_SPLIT if q >= total - ntail else SPLIT)
                if l == L - 1:
                    done.add(c)
                    if c in outs:
                        c0, n = outs[c]
                        assert all(j in done for j in range(c0, c0 + n))
                        o_copy(col0, c0, n, slot).start()

    def first_section():
        va_cp.wait()
        ua_cp.wait()
        b_cp.wait()
        vb_cp.start(priority=1)
        ub_cp.start(priority=1)
        xb_cp.start(priority=1)
        for l in range(LS):
            pre_v(l, 5)
        for l in range(LS):
            pre_u(l)

        xa_cp.wait()
        x_copy(f0, 1).start(priority=1)
        compute([(l, c, c) for l in range(LS) for c in range(NA)], 0, 0, {}, 3, 2)

        vb_cp.wait()
        ub_cp.wait()
        xb_cp.wait()
        a_ticks = [(l, c, c) for l in range(LS, L) for c in range(NA)]
        ticks = []
        for r in range(L):
            ticks += [(r, c, c) for c in range(NA, first_cb)]
            ticks += a_ticks[len(a_ticks) * r // L:len(a_ticks) * (r + 1) // L]
        first_use = {}
        for t, (l, _, _) in enumerate(ticks):
            first_use.setdefault(l, t)
        hooks = {0: [functools.partial(pre_v, l, NL) for l in range(LS, L)]}
        for l in range(LS, L):
            pos = 3 if l == LS else first_use[l] - 3
            assert 0 <= pos <= first_use[l] + 3
            hooks.setdefault(pos, []).append(functools.partial(pre_u, l))
        compute(ticks, 0, 0, {ticks[-1][1]: (0, first_cb)}, 3, 3, hooks)

    body_ticks = [(l, gi * G + j, (gi % 2) * G + j) for gi in range(NG) for l in range(L) for j in range(G)]
    body_outs = {gi * G + G - 1: (gi * G, G) for gi in range(NG - 1)}
    body_outs.update({c: (c, 1) for c in range((NG - 1) * G, NG * G)})

    def body(i, carry):
        pl.when(i == 0)(first_section)
        slot = (i + 1) & 1
        col0 = pl.multiple_of(f0 + i * bt, LANES)
        x_copy(col0, slot).wait()

        @pl.when(i == 1)
        def _():
            o_copy(0, 0, first_cb, slot).wait()

        @pl.when(i >= 2)
        def _():
            o_copy(0, 0, body_cb, slot).wait()

        @pl.when(i + 1 < nbody)
        def _():
            x_copy(col0 + bt, 1 - slot).start()

        compute(body_ticks, col0, slot, body_outs, 2, 3)
        return carry

    lax.fori_loop(0, nbody, body, 0)
    o_copy(0, 0, body_cb, (nbody - 1) % 2).wait()
    o_copy(0, 0, body_cb, nbody % 2).wait()


@jax.jit
def pallas_standalone__cross_network_dcn_v2__recsys_kernel(
    x0: jax.Array,
    U: jax.Array,
    V: jax.Array,
    bs: jax.Array,
):
    B, D = x0.shape
    L, _, R = U.shape
    bt = G * NG * LANES
    nslot = max(NA + NB, 2 * G)
    out_t = pl.pallas_call(
        _kernel,
        in_specs=[pl.BlockSpec(memory_space=pl.ANY)] * 4,
        out_specs=pl.BlockSpec(memory_space=pl.ANY),
        out_shape=jax.ShapeDtypeStruct((D, B), x0.dtype),
        scratch_shapes=[
            pltpu.VMEM((2, D, bt), BF16),
            pltpu.VMEM((2, D, bt), BF16),
            pltpu.VMEM(U.shape, BF16),
            pltpu.VMEM(V.shape, BF16),
            pltpu.VMEM(bs.shape, BF16),
            pltpu.VMEM((L, D, LANES), BF16),
            pltpu.VMEM((L, D // LANES, R, LANES), F32),
            pltpu.VMEM((L, NL, R, LANES), F32),
            pltpu.VMEM((nslot, D, LANES), F32),
            pltpu.VMEM((nslot, D, LANES), F32),
            pltpu.SemaphoreType.DMA((7,)),
            pltpu.SemaphoreType.DMA((2,)),
            pltpu.SemaphoreType.DMA((2,)),
        ],
        compiler_params=pltpu.CompilerParams(
            vmem_limit_bytes=64 * 1024 * 1024,
            disable_bounds_checks=True,
            disable_semaphore_checks=True,
        ),
    )(x0.T, U, V, bs)
    return out_t.T
```

```python
import functools

import jax
import jax.numpy as jnp
from jax import lax
from jax.experimental import pallas as pl
from jax.experimental.pallas import tpu as pltpu

F32 = jnp.float32
BF16 = jnp.bfloat16

LANES = 128
NA = 6
NB = 2
LS = 2
G = 5
NG = 6
SPLIT = 2
TAIL_SPLIT = 4
NL = 9

_dot = functools.partial(jnp.dot, preferred_element_type=F32, precision=lax.Precision.DEFAULT)


def _kernel(x_hbm, u_hbm, v_hbm, b_hbm, o_hbm, xbuf, obuf, u_ref, v_ref, b_ref,
            uz_ref, vm_ref, vb_ref, x0f_ref, xf_ref, wsem, xsem, osem):
    L, D, R = u_ref.shape
    B = x_hbm.shape[1]
    first_cb = NA + NB
    body_cb = G * NG
    bt = body_cb * LANES
    f0 = first_cb * LANES
    nbody = (B - f0) // bt
    KM = (D // LANES) * LANES
    KR = D - KM
    assert f0 + nbody * bt == B and nbody >= 2
    assert KR == 32 and R + KR - 8 == LANES and L <= 8 and 0 < LS < L

    def x_copy(col0, slot):
        return pltpu.make_async_copy(x_hbm.at[:, pl.ds(col0, bt)], xbuf.at[slot], xsem.at[slot])

    def o_copy(col0, c0, n, slot):
        w = n * LANES
        return pltpu.make_async_copy(obuf.at[slot, :, pl.ds(c0 * LANES, w)],
                                     o_hbm.at[:, pl.ds(col0 + c0 * LANES, w)], osem.at[slot])

    cols_a = pl.ds(0, NA * LANES)
    cols_b = pl.ds(NA * LANES, NB * LANES)
    va_cp = pltpu.make_async_copy(v_hbm.at[0:LS], v_ref.at[0:LS], wsem.at[0])
    ua_cp = pltpu.make_async_copy(u_hbm.at[0:LS], u_ref.at[0:LS], wsem.at[1])
    xa_cp = pltpu.make_async_copy(x_hbm.at[:, cols_a], xbuf.at[0, :, cols_a], wsem.at[2])
    vb_cp = pltpu.make_async_copy(v_hbm.at[LS:L], v_ref.at[LS:L], wsem.at[3])
    ub_cp = pltpu.make_async_copy(u_hbm.at[LS:L], u_ref.at[LS:L], wsem.at[4])
    xb_cp = pltpu.make_async_copy(x_hbm.at[:, cols_b], xbuf.at[0, :, cols_b], wsem.at[5])
    b_cp = pltpu.make_async_copy(b_hbm, b_ref, wsem.at[6])
    va_cp.start()
    ua_cp.start()
    b_cp.start()
    xa_cp.start(priority=1)

    def left_pos(l, k):
        return k if k < 8 else 8 + l

    def pre_v(l, nxlu):
        rk = lax.broadcasted_iota(jnp.int32, (KR, LANES), 0)
        for kt in range(KM // LANES):
            vm_ref[l, kt] = v_ref[l, :, kt * LANES:(kt + 1) * LANES].astype(F32)
        vr = v_ref[l, :, KM:D].astype(F32)
        for k in range(NL):
            p = left_pos(l, k)
            if k < nxlu:
                vb_ref[l, k] = jnp.broadcast_to(vr[:, p:p + 1], (R, LANES))
            else:
                vb_ref[l, k] = _dot(vr, jnp.where(rk == p, 1.0, 0.0))

    def pre_u(l):
        vzt = v_ref[l, :, KM:D].astype(F32).T[8:]
        pt = lax.dot_general(vzt, u_ref[l], (((1,), (1,)), ((), ())), preferred_element_type=F32,
                             precision=lax.Precision.DEFAULT)
        rowi = lax.broadcasted_iota(jnp.int32, (8, D), 0)
        top = jnp.where(rowi == l, b_ref[l:l + 1, :].astype(F32), pt[:8])
        p = jnp.concatenate([jnp.zeros((R, D), F32), top, pt[8:]], axis=0).T
        uz = jnp.concatenate([u_ref[l].astype(F32), p[:, R:]], axis=1)
        uz_ref[l, KR:, :] = uz[:KM].astype(BF16)
        uz_ref[l, 0:KR, :] = uz[KM:].astype(BF16)

    sub = lax.broadcasted_iota(jnp.int32, (8, LANES), 0)

    def cs(c):
        return slice(c * LANES, (c + 1) * LANES)

    def compute(ticks, col0, slot, outs, skew, ntail, hooks=None):
        x0_ref = xbuf.at[slot]
        o_ref = obuf.at[slot]
        zs = {}
        hooks = hooks or {}

        def stage_mm1(l, c, s):
            src = x0f_ref if l == 0 else xf_ref
            acc = None
            for k in range(NL):
                p = left_pos(l, k)
                t = vb_ref[l, k] * src[s, p:p + 1, :]
                acc = t if acc is None else acc + t
            for kt in range(KM // LANES):
                if l == 0:
                    xb = x0_ref[kt * LANES:(kt + 1) * LANES, cs(c)]
                else:
                    xb = xf_ref[s, KR + kt * LANES:KR + (kt + 1) * LANES, :].astype(BF16)
                acc = acc + _dot(vm_ref[l, kt], xb)
            ones_row = jnp.where(sub == l, 1.0, src[s, 8:16, :])
            zs[c] = jnp.concatenate([acc, ones_row, src[s, 16:KR, :]], axis=0).astype(BF16)

        def stage_mm2(l, c, s, nsplit):
            bounds = [((D // 16) * j // nsplit) * 16 for j in range(nsplit + 1)]
            for r0, r1 in zip(bounds[:-1], bounds[1:]):
                y = _dot(uz_ref[l, r0:r1, :], zs[c])
                x0 = x0f_ref[s, r0:r1, :]
                x = x0 if l == 0 else xf_ref[s, r0:r1, :]
                xn = x0 * y + x
                if l < L - 1:
                    xf_ref[s, r0:r1, :] = xn
                elif r0 == 0:
                    o_ref[KM:D, cs(c)] = xn[:KR].astype(BF16)
                    o_ref[0:r1 - KR, cs(c)] = xn[KR:].astype(BF16)
                else:
                    o_ref[r0 - KR:r1 - KR, cs(c)] = xn.astype(BF16)

        total = len(ticks)
        done = set()
        for t in range(total + skew):
            for h in hooks.get(t, ()):
                h()
            if t < total:
                l, c, s = ticks[t]
                assert all(ticks[q][2] != s for q in range(max(t - skew, 0), t))
                if l == 0:
                    x0f_ref[s, 0:KR, :] = x0_ref[KM:D, cs(c)].astype(F32)
                    x0f_ref[s, KR:D, :] = x0_ref[0:KM, cs(c)].astype(F32)
                stage_mm1(l, c, s)
            q = t - skew
            if q >= 0:
                l, c, s = ticks[q]
                stage_mm2(l, c, s, TAIL_SPLIT if q >= total - ntail else SPLIT)
                if l == L - 1:
                    done.add(c)
                    if c in outs:
                        c0, n = outs[c]
                        assert all(j in done for j in range(c0, c0 + n))
                        o_copy(col0, c0, n, slot).start()

    def first_section():
        va_cp.wait()
        ua_cp.wait()
        b_cp.wait()
        vb_cp.start(priority=1)
        ub_cp.start(priority=1)
        xb_cp.start(priority=1)
        for l in range(LS):
            pre_v(l, 5)
        for l in range(LS):
            pre_u(l)

        xa_cp.wait()
        x_copy(f0, 1).start(priority=1)
        compute([(l, c, c) for l in range(LS) for c in range(NA)], 0, 0, {}, 3, 2)

        vb_cp.wait()
        ub_cp.wait()
        xb_cp.wait()
        a_ticks = [(l, c, c) for l in range(LS, L) for c in range(NA)]
        ticks = []
        for r in range(L):
            ticks += [(r, c, c) for c in range(NA, first_cb)]
            ticks += a_ticks[len(a_ticks) * r // L:len(a_ticks) * (r + 1) // L]
        first_use = {}
        for t, (l, _, _) in enumerate(ticks):
            first_use.setdefault(l, t)
        hooks = {0: [functools.partial(pre_v, l, NL) for l in range(LS, L)]}
        for l in range(LS, L):
            pos = 3 if l == LS else first_use[l] - 3
            assert 0 <= pos <= first_use[l] + 3
            hooks.setdefault(pos, []).append(functools.partial(pre_u, l))
        compute(ticks, 0, 0, {ticks[-1][1]: (0, first_cb)}, 3, 3, hooks)

    body_ticks = [(l, gi * G + j, (gi % 2) * G + j) for gi in range(NG) for l in range(L) for j in range(G)]
    body_outs = {gi * G + G - 1: (gi * G, G) for gi in range(NG - 1)}
    body_outs.update({c: (c, 1) for c in range((NG - 1) * G, NG * G)})

    def body(i, carry):
        pl.when(i == 0)(first_section)
        slot = (i + 1) & 1
        col0 = pl.multiple_of(f0 + i * bt, LANES)
        x_copy(col0, slot).wait()

        @pl.when(i == 1)
        def _():
            o_copy(0, 0, first_cb, slot).wait()

        @pl.when(i >= 2)
        def _():
            o_copy(col0 - 2 * bt, 0, body_cb, slot).wait()

        @pl.when(i + 1 < nbody)
        def _():
            x_copy(col0 + bt, 1 - slot).start()

        compute(body_ticks, col0, slot, body_outs, 2, 3)
        return carry

    lax.fori_loop(0, nbody, body, 0)
    o_copy(B - 2 * bt, 0, body_cb, (nbody - 1) % 2).wait()
    o_copy(B - bt, 0, body_cb, nbody % 2).wait()


@jax.jit
def pallas_standalone__cross_network_dcn_v2__recsys_kernel(
    x0: jax.Array,
    U: jax.Array,
    V: jax.Array,
    bs: jax.Array,
):
    B, D = x0.shape
    L, _, R = U.shape
    bt = G * NG * LANES
    nslot = max(NA + NB, 2 * G)
    out_t = pl.pallas_call(
        _kernel,
        in_specs=[pl.BlockSpec(memory_space=pl.ANY)] * 4,
        out_specs=pl.BlockSpec(memory_space=pl.ANY),
        out_shape=jax.ShapeDtypeStruct((D, B), x0.dtype),
        scratch_shapes=[
            pltpu.VMEM((2, D, bt), BF16),
            pltpu.VMEM((2, D, bt), BF16),
            pltpu.VMEM(U.shape, BF16),
            pltpu.VMEM(V.shape, BF16),
            pltpu.VMEM(bs.shape, BF16),
            pltpu.VMEM((L, D, LANES), BF16),
            pltpu.VMEM((L, D // LANES, R, LANES), F32),
            pltpu.VMEM((L, NL, R, LANES), F32),
            pltpu.VMEM((nslot, D, LANES), F32),
            pltpu.VMEM((nslot, D, LANES), F32),
            pltpu.SemaphoreType.DMA((7,)),
            pltpu.SemaphoreType.DMA((2,)),
            pltpu.SemaphoreType.DMA((2,)),
        ],
        compiler_params=pltpu.CompilerParams(
            vmem_limit_bytes=64 * 1024 * 1024,
            disable_bounds_checks=True,
            disable_semaphore_checks=True,
        ),
    )(x0.T, U, V, bs)
    return out_t.T
```
